```python
import os as _os
_os.environ.setdefault("JAX_PLATFORMS", "cpu")
import jax
import jax.numpy as jnp

def _softmax(x, axis=-1):
    return jax.nn.softmax(x, axis=axis)
def _gelu(x):
    return jax.nn.gelu(x, approximate=True)
def _silu(x):
    return jax.nn.silu(x)
def _sigmoid(x):
    return jax.nn.sigmoid(x)
def _layernorm(x, axis=-1, eps=1e-5):
    m = jnp.mean(x, axis=axis, keepdims=True)
    v = jnp.var(x, axis=axis, keepdims=True)
    return (x - m) / jnp.sqrt(v + eps)
def _scatter_add(tgt, idx, src, axis=0):
    return tgt.at[idx].add(src)
def _segment_sum(src, seg, n):
    return jax.ops.segment_sum(src, seg, n)
class _Rng:
    def __init__(self, key):
        self._k = key
    def _next(self):
        self._k, sub = jax.random.split(self._k)
        return sub
    def normal(self, shape):
        return jax.random.normal(self._next(), shape, dtype=jnp.bfloat16)
    def randint(self, lo, hi, shape):
        return jax.random.randint(self._next(), shape, lo, hi, dtype=jnp.int32)
    def uniform(self, shape, lo=0.0, hi=1.0):
        return jax.random.uniform(self._next(), shape, jnp.bfloat16, lo, hi)
    def permutation(self, n):
        return jax.random.permutation(self._next(), n)


kernel_name = 'standalone__gqa_softmax__decode'

def setup_inputs():
    _rng = _Rng(jax.random.key(int.from_bytes(__import__("os").urandom(4), "little")))
    _w = (lambda a: (lambda t: t.astype(jnp.bfloat16) if jnp.issubdtype(t.dtype, jnp.floating) else t)(jnp.asarray(a)))
    B, Hq, Hkv, Sq, Sk, D = 8, 32, 32, 1, 4096, 128
    return {
        "q": _w((lambda *s: _rng.normal(s) * 0.4)(B, Hq, Sq, D)),
        "k": _w((lambda *s: _rng.normal(s) * 0.4)(B, Hkv, Sk, D)),
        "v": _w((lambda *s: _rng.normal(s) * 0.05)(B, Hkv, Sk, D)),
    }

def reference(q, k, v):
    B, Hq, Sq, D = q.shape
    Hkv = k.shape[1]
    rep = Hq // Hkv
    k = jnp.repeat(k, rep, axis=1)
    v = jnp.repeat(v, rep, axis=1)
    scale = D ** -0.5
    scores = jnp.einsum("bhqd,bhkd->bhqk", q, k) * scale
    p = _softmax(scores, axis=-1)
    return jnp.einsum("bhqk,bhkd->bhqd", p, v)
```

```python
import functools

import jax
import jax.numpy as jnp
from jax import lax
from jax.experimental import pallas as pl
from jax.experimental.pallas import tpu as pltpu

HEADS = 8
CHUNK = 128
PART = 512
NBUF = 4


def _kernel(q_hbm, k_hbm, v_hbm, o_hbm, kbuf, vbuf, qbuf, q32, obuf, o16, sems, iosem,
            *, seq, nheads, scale):
    nparts = seq // PART
    ngroups = nheads // HEADS
    niter = ngroups * nparts

    def start(grp, part, slot):
        for c in range(PART // CHUNK):
            for j in range(HEADS):
                row = (grp * HEADS + j) * seq + part * PART + c * CHUNK
                dst = pl.ds(c * CHUNK, CHUNK)
                pltpu.make_async_copy(k_hbm.at[pl.ds(row, CHUNK)], kbuf.at[slot, j, dst],
                                      sems.at[0, slot]).start(priority=0)
                pltpu.make_async_copy(v_hbm.at[pl.ds(row, CHUNK)], vbuf.at[slot, j, dst],
                                      sems.at[1, slot]).start(priority=1)

    def wait_k(slot):
        pltpu.make_async_copy(kbuf.at[slot], kbuf.at[slot], sems.at[0, slot]).wait()

    def wait_v(slot):
        pltpu.make_async_copy(vbuf.at[slot], vbuf.at[slot], sems.at[1, slot]).wait()

    q_copy = pltpu.make_async_copy(q_hbm, qbuf, iosem)
    q_copy.start()
    for i in range(NBUF):
        start(i // nparts, i % nparts, i)
    q_copy.wait()
    q32[...] = qbuf[...].astype(jnp.float32)

    def group(grp, carry):
        hrows = pl.ds(pl.multiple_of(grp * HEADS, HEADS), HEADS)
        q8 = q32[hrows, :].astype(jnp.bfloat16)
        m = l = acc = None
        for part in range(nparts):
            i = grp * nparts + part
            slot = part % NBUF if nparts % NBUF == 0 else i % NBUF
            wait_k(slot)
            rows = lax.broadcasted_iota(jnp.int32, (HEADS, PART), 0)
            s = None
            for h in range(HEADS):
                sh = lax.dot_general(q8, kbuf[slot, h], (((1,), (1,)), ((), ())),
                                     preferred_element_type=jnp.float32)
                s = sh if h == 0 else jnp.where(rows == h, sh, s)
            s = s * scale
            m_part = jnp.max(s, axis=1, keepdims=True)
            if part == 0:
                m_new = m_part
            else:
                m_new = jnp.maximum(m, m_part)
                alpha = jnp.exp(m - m_new)
            p = jnp.exp(s - m_new)
            l_part = jnp.sum(p, axis=1, keepdims=True)
            pb = p.astype(jnp.bfloat16)
            wait_v(slot)
            rows_o = lax.broadcasted_iota(jnp.int32, (HEADS, 128), 0)
            pv = None
            for h in range(HEADS):
                oh = jnp.dot(pb, vbuf[slot, h], preferred_element_type=jnp.float32)
                pv = oh if h == 0 else jnp.where(rows_o == h, oh, pv)
            if part == 0:
                l, acc = l_part, pv
            else:
                l, acc = alpha * l + l_part, alpha * acc + pv
            m = m_new
            nxt = i + NBUF

            @pl.when(nxt < niter)
            def _prefetch():
                start(nxt // nparts, nxt % nparts, slot)

        obuf[hrows, :] = acc / l
        return carry

    lax.fori_loop(0, ngroups, group, 0)
    o16[...] = obuf[...].astype(o16.dtype)
    o_copy = pltpu.make_async_copy(o16, o_hbm, iosem)
    o_copy.start()
    o_copy.wait()


@jax.jit
def pallas_standalone__gqa_softmax__decode_kernel(q, k, v):
    B, Hq, Sq, D = q.shape
    Hkv, Sk = k.shape[1], k.shape[2]
    assert Hq == Hkv and Sq == 1 and D == 128
    nheads = B * Hq
    assert nheads % HEADS == 0 and Sk % PART == 0 and NBUF <= (nheads // HEADS) * (Sk // PART)
    out = pl.pallas_call(
        functools.partial(_kernel, seq=Sk, nheads=nheads, scale=D ** -0.5),
        in_specs=[pl.BlockSpec(memory_space=pl.ANY)] * 3,
        out_specs=pl.BlockSpec(memory_space=pl.ANY),
        out_shape=jax.ShapeDtypeStruct((nheads, D), q.dtype),
        scratch_shapes=[
            pltpu.VMEM((NBUF, HEADS, PART, D), k.dtype),
            pltpu.VMEM((NBUF, HEADS, PART, D), v.dtype),
            pltpu.VMEM((nheads, D), q.dtype),
            pltpu.VMEM((nheads, D), jnp.float32),
            pltpu.VMEM((nheads, D), jnp.float32),
            pltpu.VMEM((nheads, D), q.dtype),
            pltpu.SemaphoreType.DMA((2, NBUF)),
            pltpu.SemaphoreType.DMA(()),
        ],
        compiler_params=pltpu.CompilerParams(vmem_limit_bytes=64 * 2 ** 20),
    )(q.reshape(nheads, D), k.reshape(nheads * Sk, D), v.reshape(nheads * Sk, D))
    return out.reshape(q.shape)
```
